```python
import os as _os
_os.environ.setdefault("JAX_PLATFORMS", "cpu")
import jax
import jax.numpy as jnp

def _softmax(x, axis=-1):
    return jax.nn.softmax(x, axis=axis)
def _gelu(x):
    return jax.nn.gelu(x, approximate=True)
def _silu(x):
    return jax.nn.silu(x)
def _sigmoid(x):
    return jax.nn.sigmoid(x)
def _layernorm(x, axis=-1, eps=1e-5):
    m = jnp.mean(x, axis=axis, keepdims=True)
    v = jnp.var(x, axis=axis, keepdims=True)
    return (x - m) / jnp.sqrt(v + eps)
def _scatter_add(tgt, idx, src, axis=0):
    return tgt.at[idx].add(src)
def _segment_sum(src, seg, n):
    return jax.ops.segment_sum(src, seg, n)
class _Rng:
    def __init__(self, key):
        self._k = key
    def _next(self):
        self._k, sub = jax.random.split(self._k)
        return sub
    def normal(self, shape):
        return jax.random.normal(self._next(), shape, dtype=jnp.bfloat16)
    def randint(self, lo, hi, shape):
        return jax.random.randint(self._next(), shape, lo, hi, dtype=jnp.int32)
    def uniform(self, shape, lo=0.0, hi=1.0):
        return jax.random.uniform(self._next(), shape, jnp.bfloat16, lo, hi)
    def permutation(self, n):
        return jax.random.permutation(self._next(), n)


kernel_name = 'concat_heads__grouped_kv_mqa__sliding_block__prompt'

def setup_inputs():
    _rng = _Rng(jax.random.key(int.from_bytes(__import__("os").urandom(4), "little")))
    _w = (lambda a: (lambda t: t.astype(jnp.bfloat16) if jnp.issubdtype(t.dtype, jnp.floating) else t)(jnp.asarray(a)))
    def _A_setup():
        B, S, D, H = 1, 2048, 1024, 32
        Dh = D // H
        return {
            "x": _w((lambda *s: _rng.normal(s) * 0.05)(B, S, D)),
            "wq": _w((lambda *s: _rng.normal(s) * 1.6)(D, H * Dh)),
            "wk": _w((lambda *s: _rng.normal(s) * 1.6)(D, Dh)),
            "wv": _w((lambda *s: _rng.normal(s) * 0.1)(D, Dh)),
            "wo": _w((lambda *s: _rng.normal(s) * 0.1)(H * Dh, D)),
        }
    _A_in = _A_setup()

    def _B_setup():
        B, S, D = 1, 2048, 1024
        return {
            "x": _w((lambda *s: _rng.normal(s) * 0.2)(B, S, D)),
            "wqkv": _w((lambda *s: _rng.normal(s) * 0.2)(D, 3 * D)),
            "wo": _w((lambda *s: _rng.normal(s) * 0.05)(D, D)),
        }
    _B_in = _B_setup()

    return {
        "A_x": _A_in["x"],
        "A_wq": _A_in["wq"],
        "A_wk": _A_in["wk"],
        "A_wv": _A_in["wv"],
        "A_wo": _A_in["wo"],
        "B_x": _B_in["x"],
        "B_wqkv": _B_in["wqkv"],
        "B_wo": _B_in["wo"],
    }

def reference(A_x, A_wq, A_wk, A_wv, A_wo, B_x, B_wqkv, B_wo):
    def _A_ref(x, wq, wk, wv, wo):
        B, S, D = x.shape
        H = 32
        Dh = D // H
        q = (lambda x, *d: x.transpose(*d))((x @ wq).reshape(B, S, H, Dh), 0, 2, 1, 3)
        k = x @ wk
        v = x @ wv
        scores = jnp.einsum("bhqd,bkd->bhqk", q, k) * (Dh ** -0.5)
        p = _softmax(scores, axis=-1)
        o = jnp.einsum("bhqk,bkd->bhqd", p, v)
        return (lambda x, *d: x.transpose(*d))(o, 0, 2, 1, 3).reshape(B, S, H * Dh) @ wo

    def _B_ref(x, wqkv, wo):
        B, S, D = x.shape
        H = 32; Dh = D // H; W = 256
        qkv = (lambda x, *d: x.transpose(*d))((x @ wqkv).reshape(B, S, 3, H, Dh), 2, 0, 3, 1, 4)
        q, k, v = qkv[0], qkv[1], qkv[2]
        scores = jnp.einsum("bhqd,bhkd->bhqk", q, k) * (Dh ** -0.5)
        idx = jnp.arange(S)
        mask = (idx[:, None] - idx[None, :] >= 0) & (idx[:, None] - idx[None, :] < W)
        scores = jnp.where(mask[None, None], scores, -1e9)
        p = _softmax(scores, axis=-1)
        o = jnp.einsum("bhqk,bhkd->bhqd", p, v)
        return (lambda x, *d: x.transpose(*d))(o, 0, 2, 1, 3).reshape(B, S, D) @ wo

    a = _A_ref(A_x, A_wq, A_wk, A_wv, A_wo)
    b = _B_ref(B_x, B_wqkv, B_wo)
    return jnp.concatenate([a, b], axis=-1)
```

```python
import functools
import math

import jax
import jax.numpy as jnp
import numpy as np
from jax import lax
from jax.experimental import pallas as pl
from jax.experimental.pallas import tpu as pltpu

S = 2048
D = 1024
H = 32
DH = 32
QB = 512
KC = 128
NK = S // KC
BF = jnp.bfloat16
F32 = jnp.float32
SCALE = float(DH ** -0.5 * math.log2(math.e))
NEG = float(-1e9 * math.log2(math.e))

NT_DIMS = (((1,), (1,)), ((), ()))
TN_DIMS = (((0,), (0,)), ((), ()))


def _dot(a, b):
    return jnp.dot(a, b, preferred_element_type=F32)


def _pace(m, d):
    return jnp.maximum(m, jnp.minimum(d, m))


def make_kernel(G=4, fine=True, LAG=4, bfine=True, qk4=True, pd=1, RX=2, apd=1, only=None, U1=1, U2=1, U3=1, U4=1):
    def kernel(xa_h, wq_h, wkT_h, wvT_h, woa_h, xb_h, wqkv_h, wob_h, out_h,
               xa, xb, wq, woa, wqkv, wob,
               wTa, wTb, QTa, VTa, Kpa, OTa, S0, S1, m0, m1,
               QTb, VTb, Kpb, OTb, Sb, oa, ob, dtab, sems):
        def cp(src, dst, i):
            return pltpu.make_async_copy(src, dst, sems.at[i])

        def xa_cp(qb):
            rows = pl.ds(pl.multiple_of(qb * QB, QB), QB)
            return cp(xa_h.at[0, rows, :], xa.at[rows, :], 16 + qb)

        c_wq = cp(wq_h, wq, 0)
        c_wk = cp(wkT_h, wTa.at[pl.ds(D, DH), :], 1)
        c_wv = cp(wvT_h, wTa.at[pl.ds(D + DH, DH), :], 2)
        c_woa = cp(woa_h, woa, 4)
        c_xb = cp(xb_h.at[0], xb, 5)
        c_wqkv = cp(wqkv_h, wqkv, 6)
        c_wob = cp(wob_h, wob, 7)
        if only is None:
            c_wq.start()
            xa_cp(0).start()
            c_wk.start()
            c_wv.start()

            dtab[...] = (lax.broadcasted_iota(jnp.int32, (KC, 128), 0)
                         - lax.broadcasted_iota(jnp.int32, (KC, 128), 1))

            c_wq.wait()
            for qb in range(1, S // QB):
                xa_cp(qb).start()
            for n in range(D // 128):
                wTa[pl.ds(128 * n, 128), :] = wq[:, pl.ds(128 * n, 128)].T
            c_wk.wait()
            c_wv.wait()

            def a_proj(qb, carry):
                xa_cp(qb).wait()
                xblk = xa[pl.ds(pl.multiple_of(qb * QB, QB), QB), :]
                r = lax.dot_general(wTa[...], xblk, NT_DIMS, preferred_element_type=F32)
                QTa[qb] = pltpu.bitcast((r[:D] * SCALE).astype(BF), jnp.int32)
                kt = r[D:D + DH].T.astype(BF)
                Kpa[pl.ds(pl.multiple_of(qb * (QB // 2), QB // 2), QB // 2), :] = pltpu.bitcast(kt, jnp.int32)
                vt = r[D + DH:].astype(BF)
                for cc in range(QB // KC):
                    VTa[qb * (QB // KC) + cc] = pltpu.bitcast(vt[:, cc * KC:(cc + 1) * KC], jnp.int32)
                return carry
            lax.fori_loop(0, S // QB, a_proj, 0, unroll=U1)
            for c in (c_woa, c_wqkv, c_xb, c_wob):
                c.start()

        if only in (None, 'A'):
            def ldk(c):
                return pltpu.bitcast(Kpa[pl.ds(c * KC // 2, KC // 2), :], BF)

            def a_w(g):
                qb = g // H
                h = g % H
                return pltpu.bitcast(QTa[qb, pl.ds(pl.multiple_of(h * (DH // 2), DH // 2), DH // 2), :], BF)

            def a_vt(c):
                return pltpu.bitcast(VTa[c], BF)

            def a_qk(W, S_w, c):
                s = _dot(ldk(c), W)
                S_w[pl.ds(c * KC, KC), :] = s
                return s

            def softmax_pv(s_ref_val, m_cur, vT, l, acc, dep):
                s = s_ref_val.reshape(KC // 8, 8, QB)
                if dep is None:
                    p = jnp.exp2(s - m_cur[None])
                else:
                    d = dep.reshape(KC // 16, 2, 8, QB)
                    ps = []
                    for j in range(KC // 16):
                        mj = _pace(m_cur, d[j, 1])
                        ps.append(jnp.exp2(s[2 * j:2 * j + 2] - mj[None]))
                    p = jnp.concatenate(ps, 0)
                for i in range(KC // 8):
                    l = l + p[i] if l is not None else p[i]
                pv = _dot(vT, p.reshape(KC, QB).astype(BF))
                acc = acc + pv if acc is not None else pv
                return l, acc

            def a_fin(l, acc, g):
                qb = g // H
                h = g % H
                inv = 1.0 / jnp.sum(l, axis=0, keepdims=True)
                OTa[qb, pl.ds(pl.multiple_of(h * DH, DH), DH), :] = (acc * inv).astype(BF)

            NG = (S // QB) * H
            W = a_w(0)
            mx = None
            for c in range(NK):
                s = a_qk(W, S0, c)
                cm = s.reshape(KC // 8, 8, QB).max(0)
                mx = cm if mx is None else jnp.maximum(mx, cm)
            m0[...] = jnp.broadcast_to(jnp.max(mx, axis=0, keepdims=True), (8, QB))

            bufs = [(S0, m0), (S1, m1)]

            def a_stage(g, gg, l, acc, first, last):
                S_r, m_r = bufs[gg % 2]
                S_w, m_w = bufs[(gg + 1) % 2]
                m_cur = m_r[...]
                if not last:
                    W = a_w(g + 1)
                mx = None
                prev = None
                hist = []
                for c in range(NK):
                    if not last:
                        s = a_qk(W, S_w, c)
                        cm = s.reshape(KC // 8, 8, QB).max(0)
                        mx = cm if mx is None else jnp.maximum(mx, cm)
                    if c == 0:
                        if not first:
                            m_prev = m_w[...]
                            l, acc = softmax_pv(S_w[pl.ds((NK - 1) * KC, KC), :], m_prev, a_vt(NK - 1), l, acc, None)
                            a_fin(l, acc, jnp.maximum(g - 1, 0))
                        l, acc = None, None
                    else:
                        l, acc = softmax_pv(S_r[pl.ds((c - 1) * KC, KC), :], m_cur, a_vt(c - 1), l, acc,
                                            prev if fine else None)
                    hist.append(s if not last else None)
                    prev = hist[-apd] if len(hist) >= apd else None
                if not last:
                    m_w[...] = jnp.broadcast_to(jnp.max(mx, axis=0, keepdims=True), (8, QB))
                return l, acc

            l, acc = a_stage(0, 0, None, None, True, False)
            l, acc = a_stage(1, 1, l, acc, False, False)

            def a_body(u, carry):
                l, acc = carry
                for gg in range(G):
                    g = 2 + G * u + gg
                    l, acc = a_stage(g, gg, l, acc, False, False)
                return l, acc
            nloop = (NG - 2 - 2) // G
            l, acc = lax.fori_loop(0, nloop, a_body, (l, acc))
            g0 = 2 + nloop * G
            for g in range(g0, NG):
                l, acc = a_stage(g, g % 2, l, acc, False, g == NG - 1)
            S_r, m_r = bufs[(NG - 1) % 2]
            l, acc = softmax_pv(S_r[pl.ds((NK - 1) * KC, KC), :], m_r[...], a_vt(NK - 1), l, acc, None)
            a_fin(l, acc, NG - 1)

        if only is None:
            c_woa.wait()
            c_wqkv.wait()

            def a_out(qb, carry):
                for nn in range(2):
                    col = pl.multiple_of((2 * qb + nn) * 128, 128)
                    wTb[pl.ds(col, 128), :] = wqkv[:, pl.ds(col, 128)].T
                    wTb[pl.ds(D + col, 128), :] = wqkv[:, pl.ds(2 * D + col, 128)].T
                r = lax.dot_general(OTa[qb], woa[...], TN_DIMS, preferred_element_type=F32)
                rows = pl.ds(pl.multiple_of(qb * QB, QB), QB)
                oa[rows, :] = r.astype(BF)
                pltpu.make_async_copy(oa.at[rows, :], out_h.at[0, rows, pl.ds(0, D)], sems.at[8 + qb]).start()
                return carry
            lax.fori_loop(0, S // QB, a_out, 0, unroll=U2)

        if only is None:
            c_xb.wait()

            def b_proj(qb, carry):
                rows = pl.ds(pl.multiple_of(qb * QB, QB), QB)
                xblk = xb[rows, :]
                r = lax.dot_general(wTb[...], xblk, NT_DIMS, preferred_element_type=F32)
                for cc in range(QB // KC):
                    QTb[qb * (QB // KC) + cc] = pltpu.bitcast((r[:D, cc * KC:(cc + 1) * KC] * SCALE).astype(BF), jnp.int32)
                    VTb[qb * (QB // KC) + cc] = pltpu.bitcast(r[D:, cc * KC:(cc + 1) * KC].astype(BF), jnp.int32)
                k = _dot(xblk, wqkv[:, pl.ds(D, D)]).astype(BF)
                for j in range(D // 128):
                    Kpb[j, pl.ds(pl.multiple_of(qb * (QB // 2), QB // 2), QB // 2), :] = pltpu.bitcast(
                        k[:, 128 * j:128 * (j + 1)], jnp.int32)
                return carry
            lax.fori_loop(0, S // QB, b_proj, 0, unroll=U3)

        if only in (None, 'B'):
            steps = []
            for i in range(NK):
                ts = [t for t in (i - 2, i - 1, i) if t >= 0]
                for t in ts:
                    steps.append((i, t, t == ts[0], t == ts[-1]))
            NS = len(steps)
            RING = LAG + RX

            def b_attn(j, carry):
                hrow = pl.multiple_of(j * 128, 128)
                hrow2 = pl.multiple_of(j * 64, 64)

                def b_w(i):
                    q = QTb[i, pl.ds(hrow2, 64), :]
                    tiles = []
                    for a in range(4):
                        parts = []
                        if a > 0:
                            parts.append(jnp.zeros((16 * a, 128), jnp.int32))
                        parts.append(q[16 * a:16 * a + 16])
                        if a < 3:
                            parts.append(jnp.zeros((48 - 16 * a, 128), jnp.int32))
                        tiles.append(jnp.concatenate(parts, 0))
                    return [pltpu.bitcast(x, BF) for x in tiles]

                def b_qk(n):
                    i, t, _, _ = steps[n]
                    kt = pltpu.bitcast(Kpb[j, pl.ds(t * KC // 2, KC // 2), :], BF)
                    ws = b_w(i)
                    if qk4:
                        ss = [_dot(kt, w) for w in ws]
                    else:
                        s = _dot(kt, jnp.concatenate(ws, 1))
                        ss = [s[:, 128 * a:128 * a + 128] for a in range(4)]
                    if t == i or t == i - 2:
                        d = dtab[...]
                        keep = (d <= 0) if t == i else (d > 0)
                        ss = [jnp.where(keep, x, NEG) for x in ss]
                    s = jnp.concatenate(ss, 1)
                    Sb[n % RING] = s
                    return s

                cmax = {}
                mfin = {}
                svals = {}
                l = None
                accs = None
                for n in range(NS + LAG):
                    if n < NS:
                        s = b_qk(n)
                        svals[n] = s
                        i, t, first, last = steps[n]
                        cm = s.reshape(KC // 8, 8, QB).max(0)
                        cmax[i] = cm if first else jnp.maximum(cmax[i], cm)
                        if last:
                            mfin[i] = jnp.broadcast_to(jnp.max(cmax[i], axis=0, keepdims=True), (8, QB))
                    k = n - LAG
                    if k >= 0:
                        i, t, first, last = steps[k]
                        m_cur = mfin[i]
                        sv = Sb[k % RING].reshape(KC // 8, 8, QB)
                        dep = svals.get(n - pd) if bfine else None
                        if dep is None:
                            p = jnp.exp2(sv - m_cur[None])
                        else:
                            d = dep.reshape(KC // 16, 2, 8, QB)
                            ps = []
                            for jj in range(KC // 16):
                                mj = _pace(m_cur, d[jj, 1])
                                ps.append(jnp.exp2(sv[2 * jj:2 * jj + 2] - mj[None]))
                            p = jnp.concatenate(ps, 0)
                        if first:
                            l = None
                        for r in range(KC // 8):
                            l = l + p[r] if l is not None else p[r]
                        p2 = p.reshape(KC, QB)
                        pvs = [_dot(pltpu.bitcast(VTb[t, pl.ds(hrow2 + 16 * a, 16), :], BF),
                                    p2[:, 128 * a:128 * a + 128].astype(BF)) for a in range(4)]
                        accs = pvs if first else [x + y for x, y in zip(accs, pvs)]
                        if last:
                            inv = 1.0 / jnp.sum(l, axis=0, keepdims=True)
                            o = jnp.concatenate([accs[a] * inv[:, 128 * a:128 * a + 128] for a in range(4)], 0)
                            OTb[i // 4, pl.ds(hrow, 128), pl.ds((i % 4) * 128, 128)] = o.astype(BF)
                return carry
            lax.fori_loop(0, D // 128, b_attn, 0)

        if only is None:
            c_wob.wait()

            def b_out(qb, carry):
                r = lax.dot_general(OTb[qb], wob[...], TN_DIMS, preferred_element_type=F32)
                rows = pl.ds(pl.multiple_of(qb * QB, QB), QB)
                ob[rows, :] = r.astype(BF)
                pltpu.make_async_copy(ob.at[rows, :], out_h.at[0, rows, pl.ds(D, D)], sems.at[12 + qb]).start()
                return carry
            lax.fori_loop(0, S // QB, b_out, 0, unroll=U4)

        if only is None:
            for qb in range(S // QB):
                rows = pl.ds(qb * QB, QB)
                pltpu.make_async_copy(oa.at[rows, :], out_h.at[0, rows, pl.ds(0, D)], sems.at[8 + qb]).wait()
                pltpu.make_async_copy(ob.at[rows, :], out_h.at[0, rows, pl.ds(D, D)], sems.at[12 + qb]).wait()
    return kernel


def build(**kw):
    kernel = make_kernel(**kw)

    def fn(A_x, A_wq, A_wk, A_wv, A_wo, B_x, B_wqkv, B_wo):
        vm = pltpu.VMEM
        LAGR = kw.get("LAG", 4) + kw.get("RX", 2)
        scratch = [
            vm((S, D), BF), vm((S, D), BF),
            vm((D, D), BF), vm((D, D), BF),
            vm((D, 3 * D), BF), vm((D, D), BF),
            vm((D + 2 * DH, D), BF), vm((2 * D, D), BF),
            vm((S // QB, D // 2, QB), jnp.int32),
            vm((NK, DH // 2, KC), jnp.int32),
            vm((S // 2, DH), jnp.int32),
            vm((S // QB, D, QB), BF),
            vm((S, QB), F32), vm((S, QB), F32),
            vm((8, QB), F32), vm((8, QB), F32),
            vm((NK, D // 2, KC), jnp.int32), vm((NK, D // 2, KC), jnp.int32),
            vm((D // 128, S // 2, 128), jnp.int32),
            vm((S // QB, D, QB), BF),
            vm((LAGR, KC, QB), F32),
            vm((S, D), BF), vm((S, D), BF),
            vm((KC, 128), jnp.int32),
            pltpu.SemaphoreType.DMA((20,)),
        ]
        hbm = pl.BlockSpec(memory_space=pltpu.HBM)
        return pl.pallas_call(
            kernel,
            out_shape=jax.ShapeDtypeStruct((1, S, 2 * D), BF),
            in_specs=[hbm] * 8,
            out_specs=hbm,
            scratch_shapes=scratch,
            compiler_params=pltpu.CompilerParams(vmem_limit_bytes=120 * 2**20),
            name="fused",
        )(A_x, A_wq, A_wk.T, A_wv.T, A_wo, B_x, B_wqkv, B_wo)
    return jax.jit(fn)


_fused = build(LAG=7, pd=3, apd=2, U2=True, U4=True)


def pallas_concat_heads__grouped_kv_mqa__sliding_block__prompt_kernel(
        A_x, A_wq, A_wk, A_wv, A_wo, B_x, B_wqkv, B_wo):
    return _fused(A_x, A_wq, A_wk, A_wv, A_wo, B_x, B_wqkv, B_wo)


pallas_concat_heads__grouped_kv_mqa__sliding_block__prompt_kernel = jax.jit(
    pallas_concat_heads__grouped_kv_mqa__sliding_block__prompt_kernel)
```

```python
import math

import jax
import jax.numpy as jnp
from jax import lax
from jax.experimental import pallas as pl
from jax.experimental.pallas import tpu as pltpu

S = 2048
D = 1024
H = 32
DH = 32
QB = 512
KC = 128
NK = S // KC
BF, F32, I32 = jnp.bfloat16, jnp.float32, jnp.int32
LOG2E = math.log2(math.e)
SCALE = float(DH ** -0.5 * LOG2E)
NEG = float(-1e9 * LOG2E)

A_UNROLL = 12
A_OFF, A_GR = 24, 4
B_LAG, B_RING = 6, 9
B_OFF, B_GR = 12, 2
B_OUT_ROWS = (512, 512, 512, 256, 128, 128)

NT_DIMS = (((1,), (1,)), ((), ()))
TN_DIMS = (((0,), (0,)), ((), ()))


def _dot(a, b):
    return jnp.dot(a, b, preferred_element_type=F32)


def _pack(x):
    return pltpu.bitcast(x, I32)


def _unpack(x):
    return pltpu.bitcast(x, BF)


def _pace(m, d):
    return jnp.maximum(m, jnp.minimum(d, m))


def _tree_sum(vals):
    vals = list(vals)
    while len(vals) > 1:
        nxt = [vals[i] + vals[i + 1] for i in range(0, len(vals) - 1, 2)]
        if len(vals) % 2:
            nxt.append(vals[-1])
        vals = nxt
    return vals[0]


def _lanes(x, a, n=1):
    return x[..., 128 * a:128 * (a + n)]


def _colmax8(s):
    return s.reshape(s.shape[0] // 8, 8, s.shape[1]).max(0)


def _col_max(mx):
    return jnp.broadcast_to(jnp.max(mx, axis=0, keepdims=True), mx.shape)


def _swap(x):
    return pltpu.roll(x, 64, 1)


def _lane_lo(rows):
    return lax.broadcasted_iota(I32, (rows, 128), 1) < 64


def _kernel(xa_h, wq_h, wkT_h, wvT_h, woa_h, xb_h, wqkv_h, wob_h, out_h,
            xa, xb, wq, woa, wqkv, wob,
            wTa, wTb, QTa, VTa, Kpa, OTa, S0, S1, m0, m1,
            QTb, VTb, Kpb, OTb, Sb, mb, oa, ob, dtab, dtab2, sems):

    def cp(src, dst, i):
        return pltpu.make_async_copy(src, dst, sems.at[i])

    def xa_cp(qb):
        rows = pl.ds(pl.multiple_of(qb * QB, QB), QB)
        return cp(xa_h.at[0, rows, :], xa.at[rows, :], 12 + qb)

    def xb_cp(r0, nr, i):
        rows = pl.ds(r0 if isinstance(r0, int) else pl.multiple_of(r0, QB), nr)
        return cp(xb_h.at[0, rows, :], xb.at[rows, :], i)

    def wkb_cp(c0, nc, i):
        cols = pl.ds(D + c0, nc)
        return cp(wqkv_h.at[:, cols], wqkv.at[:, cols], i)

    def oa_cp(qb):
        rows = pl.ds(qb * QB, QB)
        return cp(oa.at[rows, :], out_h.at[0, rows, pl.ds(0, D)], 16 + qb)

    def ob_cp(r0, nr, i):
        rows = pl.ds(r0, nr)
        return cp(ob.at[rows, :], out_h.at[0, rows, pl.ds(D, D)], 40 + i)

    c_wq = cp(wq_h, wq, 0)
    c_wk = cp(wkT_h, wTa.at[pl.ds(0, DH), :], 1)
    c_wv = cp(wvT_h, wTa.at[pl.ds(DH, DH), :], 2)
    c_woa = cp(woa_h, woa, 4)
    c_wqb = cp(wqkv_h.at[:, pl.ds(0, D)], wqkv.at[:, pl.ds(0, D)], 5)
    c_wvb = cp(wqkv_h.at[:, pl.ds(2 * D, D)], wqkv.at[:, pl.ds(2 * D, D)], 6)
    c_wob = cp(wob_h, wob, 7)

    ob_blocks, r0_ = [], 0
    for nr_ in B_OUT_ROWS:
        ob_blocks.append((r0_, nr_))
        r0_ += nr_
    assert r0_ == S

    steps = []
    for i in range(NK):
        ts = [t for t in (i - 2, i - 1, i) if t >= 0]
        steps += [(i, t, t == ts[0], t == ts[-1]) for t in ts]
    NS = len(steps)
    NCAR = B_LAG // 3
    assert NS % B_RING == 0 and B_LAG % 3 == 0 and B_LAG + 3 <= B_RING

    pieces = [('x', 0, 256), ('w', 0, 256), ('w', 256, 256), ('x', 256, 256), ('w', 512, 256), ('w', 768, 256)]
    descs = [xb_cp(o, sz, 24 + n) if kind == 'x' else wkb_cp(o, sz, 24 + n)
             for n, (kind, o, sz) in enumerate(pieces)]
    descs.append(xb_cp(QB, QB, 9))
    rest = [c_wq, xb_cp(2 * QB, QB, 10), xb_cp(3 * QB, QB, 11), c_wk, c_wv]
    rest += [xa_cp(qb) for qb in range(S // QB)] + [c_woa, c_wqb, c_wvb, c_wob]
    for d in descs + rest:
        d.start()

    dtab[...] = lax.broadcasted_iota(I32, (KC, 128), 0) - lax.broadcasted_iota(I32, (KC, 128), 1)
    dtab2[...] = lax.broadcasted_iota(I32, (64, 128), 0) - (lax.broadcasted_iota(I32, (64, 128), 1) & 63)
    S1[pl.ds((NK - 1) * KC, KC), :] = jnp.zeros((KC, QB), F32)
    m1[...] = jnp.zeros((8, QB), F32)
    for k in range(NS - B_LAG, NS):
        Sb[k % B_RING] = jnp.zeros((KC, QB), F32)
    mb[...] = jnp.zeros((NCAR, 8, 2 * QB), F32)

    def k_block(r0, nr, c0, nc):
        k = _dot(xb[pl.ds(r0, nr), :], wqkv[:, pl.ds(D + c0, nc)]).astype(BF)
        for j in range(nc // 128):
            Kpb[c0 // 128 + j, pl.ds(r0 // 2, nr // 2), :] = _pack(_lanes(k, j))

    xs, ws = [], []
    for (kind, o, sz), d in zip(pieces, descs):
        d.wait()
        if kind == 'x':
            xs.append((o, sz))
            if ws:
                k_block(o, sz, ws[0][0], sum(w[1] for w in ws))
        else:
            ws.append((o, sz))
            if xs:
                k_block(xs[0][0], sum(x[1] for x in xs), o, sz)
    descs[-1].wait()
    k_block(QB, QB, 0, D)
    c_wq.wait()

    def k_proj(u, carry):
        qb = u + 2
        r0 = pl.multiple_of(qb * QB, QB)
        xb_cp(r0, QB, 10 + u).wait()
        k = _dot(xb[pl.ds(r0, QB), :], wqkv[:, pl.ds(D, D)]).astype(BF)
        for j in range(D // 128):
            Kpb[j, pl.ds(pl.multiple_of(qb * (QB // 2), QB // 2), QB // 2), :] = _pack(_lanes(k, j))
        for nn in range(4):
            col = pl.multiple_of((4 * u + nn) * 128, 128)
            wTa[pl.ds(2 * DH + col, 128), :] = wq[:, pl.ds(col, 128)].T
        return carry
    lax.fori_loop(0, 2, k_proj, 0)

    c_wk.wait()
    c_wv.wait()

    def a_proj(qb, carry):
        xa_cp(qb).wait()
        xblk = xa[pl.ds(pl.multiple_of(qb * QB, QB), QB), :]
        r = lax.dot_general(wTa[...], xblk, NT_DIMS, preferred_element_type=F32)
        kt = r[:DH].T.astype(BF)
        Kpa[pl.ds(pl.multiple_of(qb * (QB // 2), QB // 2), QB // 2), :] = _pack(kt)
        vt = r[DH:2 * DH].astype(BF)
        for cc in range(QB // KC):
            VTa[qb * (QB // KC) + cc] = _pack(_lanes(vt, cc))
        QTa[qb] = _pack((r[2 * DH:] * SCALE).astype(BF))
        return carry
    lax.fori_loop(0, S // QB, a_proj, 0)

    NG = (S // QB) * H
    bufs = [(S0, m0), (S1, m1)]

    def a_rows(g):
        return pl.ds(pl.multiple_of((g % H) * (DH // 2), DH // 2), DH // 2)

    def a_w(g):
        return _unpack(QTa[g // H, a_rows(g), :])

    def a_qk(W, S_w, c):
        s = _dot(_unpack(Kpa[pl.ds(c * KC // 2, KC // 2), :]), W)
        S_w[pl.ds(c * KC, KC), :] = s
        return s

    def a_pv(S_r, c, m, l, acc, toks, base):
        s = S_r[pl.ds(c * KC, KC), :].reshape(KC // 8, 8, QB)
        ps, cache = [], {}
        for j in range(KC // 16):
            k = (base + j - A_OFF + 1) // A_GR * A_GR - 1
            if k in toks:
                if k not in cache:
                    cache[k] = _pace(m, toks[k])
                mj = cache[k]
            else:
                mj = m
            ps.append(jnp.exp2(s[2 * j:2 * j + 2] - mj[None]))
        p = jnp.concatenate(ps, 0)
        t = _tree_sum([p[i] for i in range(KC // 8)])
        l = l + t if l is not None else t
        pv = _dot(_unpack(VTa[c]), p.reshape(KC, QB).astype(BF))
        acc = acc + pv if acc is not None else pv
        return l, acc

    def a_fin(l, acc, g):
        inv = 1.0 / jnp.sum(l, axis=0, keepdims=True)
        OTa[g // H, a_rows(g), :] = _pack((acc * inv).astype(BF))

    def a_stage(g, gg, l, acc, last, toks, t0):
        S_r, m_r = bufs[gg % 2]
        S_w, m_w = bufs[(gg + 1) % 2]
        m_cur = _col_max(m_r[...])
        if not last:
            W = a_w(g + 1)
        mx = None
        for c in range(NK):
            if not last:
                s = a_qk(W, S_w, c)
                cm = _colmax8(s)
                mx = cm if mx is None else jnp.maximum(mx, cm)
                s4 = s.reshape(KC // 16, 2, 8, QB)
                for jj in range(KC // 16):
                    toks[t0 + 8 * c + jj] = s4[jj, 1]
            if c == 0:
                l, acc = a_pv(S_w, NK - 1, _col_max(m_w[...]), l, acc, toks, t0)
                a_fin(l, acc, max(g - 1, 0) if isinstance(g, int) else jnp.maximum(g - 1, 0))
                l, acc = None, None
            else:
                l, acc = a_pv(S_r, c - 1, m_cur, l, acc, toks, t0 + 8 * c)
        if not last:
            m_w[...] = mx
        return l, acc

    W = a_w(0)
    mx = None
    for c in range(NK):
        cm = _colmax8(a_qk(W, S0, c))
        mx = cm if mx is None else jnp.maximum(mx, cm)
    m0[...] = mx

    def a_body(u, carry):
        l, acc = carry
        toks = {}
        for gg in range(A_UNROLL):
            l, acc = a_stage(A_UNROLL * u + gg, gg, l, acc, False, toks, gg * 8 * NK)
        return l, acc
    nloop = (NG - 1) // A_UNROLL
    l_a, acc_a = lax.fori_loop(0, nloop, a_body, (jnp.ones((8, QB), F32), jnp.zeros((DH, QB), F32)))
    g0 = nloop * A_UNROLL
    toks1 = {}
    for g in range(g0, NG - 1):
        l_a, acc_a = a_stage(g, g % 2, l_a, acc_a, False, toks1, (g - g0) * 8 * NK)

    def a_epilogue(l, acc):
        g = NG - 1
        l, acc = a_stage(g, g % 2, l, acc, True, toks1, (g - g0) * 8 * NK)
        S_r, m_r = bufs[g % 2]
        l, acc = a_pv(S_r, NK - 1, _col_max(m_r[...]), l, acc, {}, 0)
        a_fin(l, acc, g)

    c_woa.wait()
    c_wqb.wait()
    c_wvb.wait()
    for qb in range(S // QB):
        for nn in range(2):
            col = (2 * qb + nn) * 128
            wTb[pl.ds(col, 128), :] = wqkv[:, pl.ds(col, 128)].T
            wTb[pl.ds(D + col, 128), :] = wqkv[:, pl.ds(2 * D + col, 128)].T
        r = lax.dot_general(_unpack(OTa[qb]), woa[...], TN_DIMS, preferred_element_type=F32)
        oa[pl.ds(qb * QB, QB), :] = r.astype(BF)
        oa_cp(qb).start()
        if qb == 0:
            a_epilogue(l_a, acc_a)

    def b_proj(qb, carry):
        xblk = xb[pl.ds(pl.multiple_of(qb * QB, QB), QB), :]
        r = lax.dot_general(wTb[...], xblk, NT_DIMS, preferred_element_type=F32)
        for cc in range(QB // KC):
            QTb[qb * (QB // KC) + cc] = _pack((_lanes(r[:D], cc) * SCALE).astype(BF))
            VTb[qb * (QB // KC) + cc] = _pack(_lanes(r[D:], cc).astype(BF))
        return carry
    lax.fori_loop(0, S // QB, b_proj, 0, unroll=2)

    PK = KC // 2
    qk_plan = []
    for i in range(NK):
        if i == 0:
            qk_plan.append((i, ('edge', 'pack')))
        elif i == 1:
            qk_plan += [(i, ('mid',)), (i, ('edge', 'pack'))]
        else:
            qk_plan += [(i, (k_,)) for k_ in ('mid', 'edge', 'pack')]
    assert len(qk_plan) == NS
    slot_of = {(i, k_): n % B_RING for n, (i, kinds) in enumerate(qk_plan) for k_ in kinds}

    def b_wfull(q):
        tiles = []
        for a in range(4):
            parts = []
            if a > 0:
                parts.append(jnp.zeros((16 * a, 128), I32))
            parts.append(q[16 * a:16 * a + 16])
            if a < 3:
                parts.append(jnp.zeros((48 - 16 * a, 128), I32))
            tiles.append(jnp.concatenate(parts, 0))
        return _unpack(jnp.concatenate(tiles, 1))

    def b_whalf(q, upper):
        lo = _lane_lo(16)
        tiles = []
        for a in (0, 2):
            qa, qb_ = q[16 * a:16 * a + 16], q[16 * a + 16:16 * a + 32]
            if upper:
                ra, rb = jnp.where(lo, _swap(qa), 0), jnp.where(lo, 0, qb_)
            else:
                ra, rb = jnp.where(lo, qa, 0), jnp.where(lo, 0, _swap(qb_))
            parts = []
            if a > 0:
                parts.append(jnp.zeros((16 * a, 128), I32))
            parts += [ra, rb]
            if a < 2:
                parts.append(jnp.zeros((32 - 16 * a, 128), I32))
            tiles.append(jnp.concatenate(parts, 0))
        return _unpack(jnp.concatenate(tiles, 1))

    def b_k(j, t, r0, nr):
        return _unpack(Kpb[j, pl.ds(t * PK + r0 // 2, nr // 2), :])

    def sel(keep, s):
        return jnp.concatenate([jnp.where(keep, _lanes(s, a), NEG) for a in range(s.shape[1] // 128)], 1)

    def b_qk(j, n, st, toks):
        i, kinds = qk_plan[n]
        q = QTb[i, pl.ds(pl.multiple_of(j * 64, 64), 64), :]
        for kind in kinds:
            slot = slot_of[(i, kind)]
            if kind == 'mid':
                s = _dot(b_k(j, i - 1, 0, KC), b_wfull(q))
                Sb[slot] = s
            elif kind == 'edge':
                d = dtab[...]
                if i >= 2:
                    kt = jnp.concatenate([b_k(j, i - 2, 64, 64), b_k(j, i, 0, 64)], 0)
                    s = _dot(kt, b_wfull(q))
                    s = jnp.concatenate([sel(d[64:] > 0, s[:64]), sel(d[:64] <= 0, s[64:])], 0)
                    Sb[slot] = s
                else:
                    s = sel(d[:64] <= 0, _dot(b_k(j, i, 0, 64), b_wfull(q)))
                    Sb[slot, pl.ds(64, 64), :] = s
            else:
                d2 = dtab2[...]
                su = sel(d2 <= 0, _dot(b_k(j, i, 64, 64), b_whalf(q, True)))
                Sb[slot, pl.ds(0, 64), pl.ds(256, 256)] = su
                st['cu'] = _colmax8(su)
                if i >= 2:
                    sl = sel(d2 > 0, _dot(b_k(j, i - 2, 0, 64), b_whalf(q, False)))
                    Sb[slot, pl.ds(0, 64), pl.ds(0, 256)] = sl
                    st['cl'] = _colmax8(sl)
                    s = jnp.concatenate([sl, su], 1)
                else:
                    st['cl'] = None
                    s = jnp.concatenate([su, su], 1)
            if kind != 'pack':
                st['cm'] = _colmax8(s) if st['cm'] is None else jnp.maximum(st['cm'], _colmax8(s))
            s4 = s.reshape(s.shape[0] // 16, 2, 8, QB)
            for jj in range(s.shape[0] // 16):
                toks[st['nt']] = s4[jj, 1]
                st['nt'] += 1

    def b_max(cm, cl, cu):
        lo = _lane_lo(8)
        heads = []
        for p in range(2):
            u = _lanes(cu, p)
            ma, mb_ = _lanes(cm, 2 * p), _lanes(cm, 2 * p + 1)
            if cl is not None:
                l_ = _lanes(cl, p)
                ea, eb = jnp.where(lo, l_, _swap(u)), jnp.where(lo, _swap(l_), u)
            else:
                ea, eb = jnp.where(lo, ma, _swap(u)), jnp.where(lo, mb_, u)
            heads += [jnp.maximum(ma, ea), jnp.maximum(mb_, eb)]
        m = _col_max(jnp.concatenate(heads, 1))
        mt = [jnp.where(lo, _lanes(m, 2 * p), _swap(_lanes(m, 2 * p + 1))) for p in range(2)]
        mu = [jnp.where(lo, _swap(_lanes(m, 2 * p)), _lanes(m, 2 * p + 1)) for p in range(2)]
        return jnp.concatenate([m] + mt + mu, 1)

    def b_exp(sv, m, toks, st):
        nr, w = sv.shape
        s3 = sv.reshape(nr // 8, 8, w)
        per = QB // w
        ps, cache = [], {}
        for jj in range(nr // 16):
            k = (st['ne'] + B_OFF + 1) // B_GR * B_GR - 1
            if k in toks:
                if k not in cache:
                    cache[k] = _pace(m, _lanes(toks[k], 0, w // 128))
                mj = cache[k]
            else:
                mj = m
            ps.append(jnp.exp2(s3[2 * jj:2 * jj + 2] - mj[None]))
            if jj % per == per - 1:
                st['ne'] += 1
        return jnp.concatenate(ps, 0)

    def acc_sum(l, p):
        t = p.sum(0)
        return l + t if l is not None else t

    def b_pv(j, k, mm, pst, toks, st):
        i, t, first, last = steps[k]
        kk = st['np']
        st['np'] += 1
        tk = st['lt'].get(kk - 3)
        if tk is not None:
            mm = _pace(mm, jnp.concatenate([tk, tk], 1))
        m = mm[:, :QB]
        lo8, lo64 = _lane_lo(8), _lane_lo(64)
        if first:
            pst['l'] = pst['ll'] = pst['lu'] = None
        if t == i - 1:
            p = b_exp(Sb[slot_of[(i, 'mid')]], m, toks, st)
            pst['l'] = acc_sum(pst['l'], p)
            p2 = p.reshape(KC, QB)
            ws = [_lanes(p2, a) for a in range(4)]
        elif t == i - 2:
            ph = b_exp(Sb[slot_of[(i, 'pack')], pl.ds(0, 64), pl.ds(0, 256)], mm[:, QB:QB + 256], toks, st)
            pe = b_exp(Sb[slot_of[(i, 'edge')], pl.ds(0, 64), :], m, toks, st)
            pst['ll'] = acc_sum(None, ph)
            pst['l'] = acc_sum(pst['l'], pe)
            ph2, pe2 = ph.reshape(64, 256), pe.reshape(64, QB)
            ws = []
            for pr in range(2):
                x = _lanes(ph2, pr)
                for a, top in ((2 * pr, jnp.where(lo64, x, 0.0)), (2 * pr + 1, jnp.where(lo64, _swap(x), 0.0))):
                    ws.append(jnp.concatenate([top, _lanes(pe2, a)], 0))
        else:
            pe = b_exp(Sb[slot_of[(i, 'edge')], pl.ds(64, 64), :], m, toks, st)
            ph = b_exp(Sb[slot_of[(i, 'pack')], pl.ds(0, 64), pl.ds(256, 256)], mm[:, QB + 256:], toks, st)
            pst['lu'] = acc_sum(None, ph)
            pst['l'] = acc_sum(pst['l'], pe)
            ph2, pe2 = ph.reshape(64, 256), pe.reshape(64, QB)
            ws = []
            for pr in range(2):
                x = _lanes(ph2, pr)
                for a, bot in ((2 * pr, jnp.where(lo64, 0.0, _swap(x))), (2 * pr + 1, jnp.where(lo64, 0.0, x))):
                    ws.append(jnp.concatenate([_lanes(pe2, a), bot], 0))
        ws = [w.astype(BF) for w in ws]
        lt = pst['l']
        for extra in (pst['ll'] if t == i - 2 else None, pst['lu'] if t == i else None):
            if extra is not None:
                lt = jnp.maximum(lt, jnp.concatenate([extra, extra], 1))
        st['lt'][kk] = lt
        vrow = j * 64
        pvs = [_dot(_unpack(VTb[t, pl.ds(pl.multiple_of(vrow + 16 * a, 16), 16), :]), ws[a]) for a in range(4)]
        pst['acc'] = pvs if first else [x + y for x, y in zip(pst['acc'], pvs)]
        if last:
            l, lu, ll = pst['l'], pst['lu'], pst['ll']
            outs, invs = [], []
            for pr in range(2):
                u = _lanes(lu, pr)
                if ll is not None:
                    w_ = _lanes(ll, pr)
                    ea, eb = jnp.where(lo8, w_, _swap(u)), jnp.where(lo8, _swap(w_), u)
                else:
                    ea, eb = jnp.where(lo8, 0.0, _swap(u)), jnp.where(lo8, 0.0, u)
                for a, e in ((2 * pr, ea), (2 * pr + 1, eb)):
                    inv = 1.0 / jnp.sum(_lanes(l, a) + e, axis=0, keepdims=True)
                    outs.append(pst['acc'][a] * inv)
                    invs.append(inv)
            st['lt'][kk] = jnp.concatenate([jnp.broadcast_to(v, (8, 128)) for v in invs], 1)
            o = jnp.concatenate(outs, 0)
            OTb[i // 4, pl.ds(pl.multiple_of(vrow, 64), 64), pl.ds((i % 4) * 128, 128)] = _pack(o.astype(BF))

    def b_iter(j, jp, do_qk):
        mfin = {}
        for c in range(NCAR):
            raw = mb[c]
            if c == NCAR - 1:
                raw = b_max(raw[:, :QB], raw[:, QB:QB + 256], raw[:, QB + 256:])
            mfin[NK - NCAR + c] = raw
        toks = {}
        st = {'nt': 0, 'ne': -20 * NCAR, 'np': 0, 'lt': {}}
        pst = {}
        for n in range(NS if do_qk else B_LAG):
            if do_qk:
                i = qk_plan[n][0]
                if n == 0 or qk_plan[n - 1][0] != i:
                    st['cm'] = st['cl'] = st['cu'] = None
                b_qk(j, n, st, toks)
                if n == NS - 1 or qk_plan[n + 1][0] != i:
                    if i == NK - 1:
                        mb[NCAR - 1] = jnp.concatenate([st['cm'], st['cl'], st['cu']], 1)
                    elif i >= NK - NCAR:
                        mb[i - (NK - NCAR)] = b_max(st['cm'], st['cl'], st['cu'])
                    else:
                        mfin[i] = b_max(st['cm'], st['cl'], st['cu'])
            k = n - B_LAG
            if k >= 0:
                b_pv(j, k, mfin[steps[k][0]], pst, toks, st)
            else:
                b_pv(jp, k + NS, mfin[steps[k + NS][0]], pst, toks, st)

    def b_body(j, carry):
        b_iter(j, jnp.maximum(j - 1, 0), True)
        return carry
    lax.fori_loop(0, D // 128, b_body, 0)

    c_wob.wait()
    for n, (r0, nr) in enumerate(ob_blocks):
        qb, off = divmod(r0, QB)
        r = lax.dot_general(_unpack(OTb[qb, :, pl.ds(off, nr)]), wob[...], TN_DIMS, preferred_element_type=F32)
        ob[pl.ds(r0, nr), :] = r.astype(BF)
        ob_cp(r0, nr, n).start()
        if n == 0:
            b_iter(None, D // 128 - 1, False)

    for qb in range(S // QB):
        oa_cp(qb).wait()
    for n, (r0, nr) in enumerate(ob_blocks):
        ob_cp(r0, nr, n).wait()


@jax.jit
def pallas_concat_heads__grouped_kv_mqa__sliding_block__prompt_kernel(
        A_x, A_wq, A_wk, A_wv, A_wo, B_x, B_wqkv, B_wo):
    vm = pltpu.VMEM
    scratch = [
        vm((S, D), BF), vm((S, D), BF),
        vm((D, D), BF), vm((D, D), BF),
        vm((D, 3 * D), BF), vm((D, D), BF),
        vm((D + 2 * DH, D), BF), vm((2 * D, D), BF),
        vm((S // QB, D // 2, QB), I32),
        vm((NK, DH // 2, KC), I32),
        vm((S // 2, DH), I32),
        vm((S // QB, D // 2, QB), I32),
        vm((S, QB), F32), vm((S, QB), F32),
        vm((8, QB), F32), vm((8, QB), F32),
        vm((NK, D // 2, KC), I32), vm((NK, D // 2, KC), I32),
        vm((D // 128, S // 2, 128), I32),
        vm((S // QB, D // 2, QB), I32),
        vm((B_RING, KC, QB), F32),
        vm((B_LAG // 3, 8, 2 * QB), F32),
        vm((S, D), BF), vm((S, D), BF),
        vm((KC, 128), I32), vm((64, 128), I32),
        pltpu.SemaphoreType.DMA((56,)),
    ]
    hbm = pl.BlockSpec(memory_space=pltpu.HBM)
    return pl.pallas_call(
        _kernel,
        out_shape=jax.ShapeDtypeStruct((1, S, 2 * D), BF),
        in_specs=[hbm] * 8,
        out_specs=hbm,
        scratch_shapes=scratch,
        compiler_params=pltpu.CompilerParams(vmem_limit_bytes=120 * 2**20),
        name="fused",
    )(A_x, A_wq, A_wk.T, A_wv.T, A_wo, B_x, B_wqkv, B_wo)
```

```python
import math

import jax
import jax.numpy as jnp
from jax import lax
from jax.experimental import pallas as pl
from jax.experimental.pallas import tpu as pltpu

S = 2048
D = 1024
H = 32
DH = 32
QB = 512
KC = 128
NK = S // KC
BF, F32, I32 = jnp.bfloat16, jnp.float32, jnp.int32
LOG2E = math.log2(math.e)
SCALE = float(DH ** -0.5 * LOG2E)
NEG = float(-1e9 * LOG2E)

A_UNROLL = 12
A_OFF, A_GR = 24, 4
B_LAG, B_RING = 6, 9
B_OFF, B_GR = 6, 2
B_OUT_ROWS = (512, 512, 512, 256, 128, 128)

NT_DIMS = (((1,), (1,)), ((), ()))
TN_DIMS = (((0,), (0,)), ((), ()))


def _dot(a, b):
    return jnp.dot(a, b, preferred_element_type=F32)


def _pack(x):
    return pltpu.bitcast(x, I32)


def _unpack(x):
    return pltpu.bitcast(x, BF)


def _pace(m, d):
    return jnp.maximum(m, jnp.minimum(d, m))


def _tree_sum(vals):
    vals = list(vals)
    while len(vals) > 1:
        nxt = [vals[i] + vals[i + 1] for i in range(0, len(vals) - 1, 2)]
        if len(vals) % 2:
            nxt.append(vals[-1])
        vals = nxt
    return vals[0]


def _lanes(x, a, n=1):
    return x[..., 128 * a:128 * (a + n)]


def _colmax8(s):
    return s.reshape(s.shape[0] // 8, 8, s.shape[1]).max(0)


def _col_max(mx):
    return jnp.broadcast_to(jnp.max(mx, axis=0, keepdims=True), mx.shape)


def _swap(x):
    return pltpu.roll(x, 64, 1)


def _lane_lo(rows):
    return lax.broadcasted_iota(I32, (rows, 128), 1) < 64


def _kernel(xa_h, wq_h, wkT_h, wvT_h, woa_h, xb_h, wqkv_h, wob_h, out_h,
            xa, xb, wq, woa, wqkv, wob,
            wTa, wTb, QTa, VTa, Kpa, OTa, S0, S1, m0, m1,
            QTb, VTb, Kpb, OTb, Sb, mb, oa, ob, dtab, dtab2, sems):

    def cp(src, dst, i):
        return pltpu.make_async_copy(src, dst, sems.at[i])

    def xa_cp(qb):
        rows = pl.ds(pl.multiple_of(qb * QB, QB), QB)
        return cp(xa_h.at[0, rows, :], xa.at[rows, :], 12 + qb)

    def xb_cp(r0, nr, i):
        rows = pl.ds(r0 if isinstance(r0, int) else pl.multiple_of(r0, QB), nr)
        return cp(xb_h.at[0, rows, :], xb.at[rows, :], i)

    def wkb_cp(c0, nc, i):
        cols = pl.ds(D + c0, nc)
        return cp(wqkv_h.at[:, cols], wqkv.at[:, cols], i)

    def oa_cp(qb):
        rows = pl.ds(qb * QB, QB)
        return cp(oa.at[rows, :], out_h.at[0, rows, pl.ds(0, D)], 16 + qb)

    def ob_cp(r0, nr, i):
        rows = pl.ds(r0, nr)
        return cp(ob.at[rows, :], out_h.at[0, rows, pl.ds(D, D)], 40 + i)

    c_wq = cp(wq_h, wq, 0)
    c_wk = cp(wkT_h, wTa.at[pl.ds(0, DH), :], 1)
    c_wv = cp(wvT_h, wTa.at[pl.ds(DH, DH), :], 2)
    c_woa = cp(woa_h, woa, 4)
    c_wqb = cp(wqkv_h.at[:, pl.ds(0, D)], wqkv.at[:, pl.ds(0, D)], 5)
    c_wvb = cp(wqkv_h.at[:, pl.ds(2 * D, D)], wqkv.at[:, pl.ds(2 * D, D)], 6)
    c_wob = cp(wob_h, wob, 7)

    ob_blocks, r0_ = [], 0
    for nr_ in B_OUT_ROWS:
        ob_blocks.append((r0_, nr_))
        r0_ += nr_
    assert r0_ == S

    steps = []
    for i in range(NK):
        ts = [t for t in (i - 2, i - 1, i) if t >= 0]
        steps += [(i, t, t == ts[0], t == ts[-1]) for t in ts]
    NS = len(steps)
    NCAR = B_LAG // 3
    assert NS % B_RING == 0 and B_LAG % 3 == 0 and B_LAG + 3 <= B_RING

    pieces = [('x', 0, 256), ('w', 0, 256), ('w', 256, 256), ('x', 256, 256), ('w', 512, 256), ('w', 768, 256)]
    descs = [xb_cp(o, sz, 24 + n) if kind == 'x' else wkb_cp(o, sz, 24 + n)
             for n, (kind, o, sz) in enumerate(pieces)]
    descs.append(xb_cp(QB, QB, 9))
    rest = [c_wq, xb_cp(2 * QB, QB, 10), xb_cp(3 * QB, QB, 11), c_wk, c_wv]
    rest += [xa_cp(qb) for qb in range(S // QB)] + [c_woa, c_wqb, c_wvb, c_wob]
    for d in descs + rest:
        d.start()

    dtab[...] = lax.broadcasted_iota(I32, (KC, 128), 0) - lax.broadcasted_iota(I32, (KC, 128), 1)
    dtab2[...] = lax.broadcasted_iota(I32, (64, 128), 0) - (lax.broadcasted_iota(I32, (64, 128), 1) & 63)
    S1[pl.ds((NK - 1) * KC, KC), :] = jnp.zeros((KC, QB), F32)
    m1[...] = jnp.zeros((8, QB), F32)
    for k in range(NS - B_LAG, NS):
        Sb[k % B_RING] = jnp.zeros((KC, QB), F32)
    mb[...] = jnp.zeros((NCAR, 8, 2 * QB), F32)

    def k_block(r0, nr, c0, nc):
        k = _dot(xb[pl.ds(r0, nr), :], wqkv[:, pl.ds(D + c0, nc)]).astype(BF)
        for j in range(nc // 128):
            Kpb[c0 // 128 + j, pl.ds(r0 // 2, nr // 2), :] = _pack(_lanes(k, j))

    xs, ws = [], []
    for (kind, o, sz), d in zip(pieces, descs):
        d.wait()
        if kind == 'x':
            xs.append((o, sz))
            if ws:
                k_block(o, sz, ws[0][0], sum(w[1] for w in ws))
        else:
            ws.append((o, sz))
            if xs:
                k_block(xs[0][0], sum(x[1] for x in xs), o, sz)
    descs[-1].wait()
    k_block(QB, QB, 0, D)
    c_wq.wait()

    def k_proj(u, carry):
        qb = u + 2
        r0 = pl.multiple_of(qb * QB, QB)
        xb_cp(r0, QB, 10 + u).wait()
        k = _dot(xb[pl.ds(r0, QB), :], wqkv[:, pl.ds(D, D)]).astype(BF)
        for j in range(D // 128):
            Kpb[j, pl.ds(pl.multiple_of(qb * (QB // 2), QB // 2), QB // 2), :] = _pack(_lanes(k, j))
        for nn in range(4):
            col = pl.multiple_of((4 * u + nn) * 128, 128)
            wTa[pl.ds(2 * DH + col, 128), :] = wq[:, pl.ds(col, 128)].T
        return carry
    lax.fori_loop(0, 2, k_proj, 0)

    c_wk.wait()
    c_wv.wait()

    def a_proj(qb, carry):
        xa_cp(qb).wait()
        xblk = xa[pl.ds(pl.multiple_of(qb * QB, QB), QB), :]
        r = lax.dot_general(wTa[...], xblk, NT_DIMS, preferred_element_type=F32)
        kt = r[:DH].T.astype(BF)
        Kpa[pl.ds(pl.multiple_of(qb * (QB // 2), QB // 2), QB // 2), :] = _pack(kt)
        vt = r[DH:2 * DH].astype(BF)
        for cc in range(QB // KC):
            VTa[qb * (QB // KC) + cc] = _pack(_lanes(vt, cc))
        QTa[qb] = _pack((r[2 * DH:] * SCALE).astype(BF))
        return carry
    lax.fori_loop(0, S // QB, a_proj, 0)

    NG = (S // QB) * H
    bufs = [(S0, m0), (S1, m1)]

    def a_rows(g):
        return pl.ds(pl.multiple_of((g % H) * (DH // 2), DH // 2), DH // 2)

    def a_w(g):
        return _unpack(QTa[g // H, a_rows(g), :])

    def a_qk(W, S_w, c):
        s = _dot(_unpack(Kpa[pl.ds(c * KC // 2, KC // 2), :]), W)
        S_w[pl.ds(c * KC, KC), :] = s
        return s

    def a_pv(S_r, c, m, l, acc, toks, base):
        s = S_r[pl.ds(c * KC, KC), :].reshape(KC // 8, 8, QB)
        ps, cache = [], {}
        for j in range(KC // 16):
            k = (base + j - A_OFF + 1) // A_GR * A_GR - 1
            if k in toks:
                if k not in cache:
                    cache[k] = _pace(m, toks[k])
                mj = cache[k]
            else:
                mj = m
            ps.append(jnp.exp2(s[2 * j:2 * j + 2] - mj[None]))
        p = jnp.concatenate(ps, 0)
        t = _tree_sum([p[i] for i in range(KC // 8)])
        l = l + t if l is not None else t
        pv = _dot(_unpack(VTa[c]), p.reshape(KC, QB).astype(BF))
        acc = acc + pv if acc is not None else pv
        return l, acc

    def a_fin(l, acc, g):
        inv = 1.0 / jnp.sum(l, axis=0, keepdims=True)
        OTa[g // H, a_rows(g), :] = _pack((acc * inv).astype(BF))

    def a_stage(g, gg, l, acc, last, toks, t0):
        S_r, m_r = bufs[gg % 2]
        S_w, m_w = bufs[(gg + 1) % 2]
        m_cur = _col_max(m_r[...])
        if not last:
            W = a_w(g + 1)
        mx = None
        for c in range(NK):
            if not last:
                s = a_qk(W, S_w, c)
                cm = _colmax8(s)
                mx = cm if mx is None else jnp.maximum(mx, cm)
                s4 = s.reshape(KC // 16, 2, 8, QB)
                for jj in range(KC // 16):
                    toks[t0 + 8 * c + jj] = s4[jj, 1]
            if c == 0:
                l, acc = a_pv(S_w, NK - 1, _col_max(m_w[...]), l, acc, toks, t0)
                a_fin(l, acc, max(g - 1, 0) if isinstance(g, int) else jnp.maximum(g - 1, 0))
                l, acc = None, None
            else:
                l, acc = a_pv(S_r, c - 1, m_cur, l, acc, toks, t0 + 8 * c)
        if not last:
            m_w[...] = mx
        return l, acc

    for c in (c_woa, c_wqb, c_wvb, c_wob):
        c.wait()

    W = a_w(0)
    mx = None
    for c in range(NK):
        cm = _colmax8(a_qk(W, S0, c))
        mx = cm if mx is None else jnp.maximum(mx, cm)
    m0[...] = mx

    def a_body(u, carry):
        l, acc = carry
        toks = {}
        for gg in range(A_UNROLL):
            l, acc = a_stage(A_UNROLL * u + gg, gg, l, acc, False, toks, gg * 8 * NK)
        return l, acc
    nloop = (NG - 1) // A_UNROLL
    l_a, acc_a = lax.fori_loop(0, nloop, a_body, (jnp.ones((8, QB), F32), jnp.zeros((DH, QB), F32)))
    g0 = nloop * A_UNROLL
    toks1 = {}
    for g in range(g0, NG - 1):
        l_a, acc_a = a_stage(g, g % 2, l_a, acc_a, False, toks1, (g - g0) * 8 * NK)

    def a_epilogue(l, acc):
        g = NG - 1
        l, acc = a_stage(g, g % 2, l, acc, True, toks1, (g - g0) * 8 * NK)
        S_r, m_r = bufs[g % 2]
        l, acc = a_pv(S_r, NK - 1, _col_max(m_r[...]), l, acc, {}, 0)
        a_fin(l, acc, g)

    for qb in range(S // QB):
        for nn in range(2):
            col = (2 * qb + nn) * 128
            wTb[pl.ds(col, 128), :] = wqkv[:, pl.ds(col, 128)].T
            wTb[pl.ds(D + col, 128), :] = wqkv[:, pl.ds(2 * D + col, 128)].T
        r = lax.dot_general(_unpack(OTa[qb]), woa[...], TN_DIMS, preferred_element_type=F32)
        if qb == 0:
            a_epilogue(l_a, acc_a)
        oa[pl.ds(qb * QB, QB), :] = r.astype(BF)
        oa_cp(qb).start()

    def b_proj(qb, carry):
        xblk = xb[pl.ds(pl.multiple_of(qb * QB, QB), QB), :]
        r = lax.dot_general(wTb[...], xblk, NT_DIMS, preferred_element_type=F32)
        for cc in range(QB // KC):
            QTb[qb * (QB // KC) + cc] = _pack((_lanes(r[:D], cc) * SCALE).astype(BF))
            VTb[qb * (QB // KC) + cc] = _pack(_lanes(r[D:], cc).astype(BF))
        return carry
    lax.fori_loop(0, S // QB, b_proj, 0, unroll=2)

    PK = KC // 2
    qk_plan = []
    for i in range(NK):
        if i == 0:
            qk_plan.append((i, ('edge', 'pack')))
        elif i == 1:
            qk_plan += [(i, ('mid',)), (i, ('edge', 'pack'))]
        else:
            qk_plan += [(i, (k_,)) for k_ in ('mid', 'edge', 'pack')]
    assert len(qk_plan) == NS
    slot_of = {(i, k_): n % B_RING for n, (i, kinds) in enumerate(qk_plan) for k_ in kinds}

    def b_wfull(q):
        tiles = []
        for a in range(4):
            parts = []
            if a > 0:
                parts.append(jnp.zeros((16 * a, 128), I32))
            parts.append(q[16 * a:16 * a + 16])
            if a < 3:
                parts.append(jnp.zeros((48 - 16 * a, 128), I32))
            tiles.append(jnp.concatenate(parts, 0))
        return _unpack(jnp.concatenate(tiles, 1))

    def b_whalf(q, upper):
        lo = _lane_lo(16)
        tiles = []
        for a in (0, 2):
            qa, qb_ = q[16 * a:16 * a + 16], q[16 * a + 16:16 * a + 32]
            if upper:
                ra, rb = jnp.where(lo, _swap(qa), 0), jnp.where(lo, 0, qb_)
            else:
                ra, rb = jnp.where(lo, qa, 0), jnp.where(lo, 0, _swap(qb_))
            parts = []
            if a > 0:
                parts.append(jnp.zeros((16 * a, 128), I32))
            parts += [ra, rb]
            if a < 2:
                parts.append(jnp.zeros((32 - 16 * a, 128), I32))
            tiles.append(jnp.concatenate(parts, 0))
        return _unpack(jnp.concatenate(tiles, 1))

    def b_k(j, t, r0, nr):
        return _unpack(Kpb[j, pl.ds(t * PK + r0 // 2, nr // 2), :])

    def sel(keep, s):
        return jnp.concatenate([jnp.where(keep, _lanes(s, a), NEG) for a in range(s.shape[1] // 128)], 1)

    def b_qk(j, n, st, toks):
        i, kinds = qk_plan[n]
        q = QTb[i, pl.ds(pl.multiple_of(j * 64, 64), 64), :]
        for kind in kinds:
            slot = slot_of[(i, kind)]
            if kind == 'mid':
                s = _dot(b_k(j, i - 1, 0, KC), b_wfull(q))
                Sb[slot] = s
            elif kind == 'edge':
                d = dtab[...]
                if i >= 2:
                    kt = jnp.concatenate([b_k(j, i - 2, 64, 64), b_k(j, i, 0, 64)], 0)
                    s = _dot(kt, b_wfull(q))
                    s = jnp.concatenate([sel(d[64:] > 0, s[:64]), sel(d[:64] <= 0, s[64:])], 0)
                    Sb[slot] = s
                else:
                    s = sel(d[:64] <= 0, _dot(b_k(j, i, 0, 64), b_wfull(q)))
                    Sb[slot, pl.ds(64, 64), :] = s
            else:
                d2 = dtab2[...]
                su = sel(d2 <= 0, _dot(b_k(j, i, 64, 64), b_whalf(q, True)))
                Sb[slot, pl.ds(0, 64), pl.ds(256, 256)] = su
                st['cu'] = _colmax8(su)
                if i >= 2:
                    sl = sel(d2 > 0, _dot(b_k(j, i - 2, 0, 64), b_whalf(q, False)))
                    Sb[slot, pl.ds(0, 64), pl.ds(0, 256)] = sl
                    st['cl'] = _colmax8(sl)
                    s = jnp.concatenate([sl, su], 1)
                else:
                    st['cl'] = None
                    s = jnp.concatenate([su, su], 1)
            if kind != 'pack':
                st['cm'] = _colmax8(s) if st['cm'] is None else jnp.maximum(st['cm'], _colmax8(s))
            s4 = s.reshape(s.shape[0] // 16, 2, 8, QB)
            for jj in range(s.shape[0] // 16):
                toks[st['nt']] = s4[jj, 1]
                st['nt'] += 1

    def b_max(cm, cl, cu):
        lo = _lane_lo(8)
        heads = []
        for p in range(2):
            u = _lanes(cu, p)
            ma, mb_ = _lanes(cm, 2 * p), _lanes(cm, 2 * p + 1)
            if cl is not None:
                l_ = _lanes(cl, p)
                ea, eb = jnp.where(lo, l_, _swap(u)), jnp.where(lo, _swap(l_), u)
            else:
                ea, eb = jnp.where(lo, ma, _swap(u)), jnp.where(lo, mb_, u)
            heads += [jnp.maximum(ma, ea), jnp.maximum(mb_, eb)]
        m = _col_max(jnp.concatenate(heads, 1))
        mt = [jnp.where(lo, _lanes(m, 2 * p), _swap(_lanes(m, 2 * p + 1))) for p in range(2)]
        mu = [jnp.where(lo, _swap(_lanes(m, 2 * p)), _lanes(m, 2 * p + 1)) for p in range(2)]
        return jnp.concatenate([m] + mt + mu, 1)

    def b_exp(sv, m, toks, st):
        nr, w = sv.shape
        s3 = sv.reshape(nr // 8, 8, w)
        per = QB // w
        ps, cache = [], {}
        for jj in range(nr // 16):
            k = (st['ne'] + B_OFF + 1) // B_GR * B_GR - 1
            if k in toks:
                if k not in cache:
                    cache[k] = _pace(m, _lanes(toks[k], 0, w // 128))
                mj = cache[k]
            else:
                mj = m
            ps.append(jnp.exp2(s3[2 * jj:2 * jj + 2] - mj[None]))
            if jj % per == per - 1:
                st['ne'] += 1
        return jnp.concatenate(ps, 0)

    def acc_sum(l, p):
        t = p.sum(0)
        return l + t if l is not None else t

    def b_pv(j, k, mm, pst, toks, st):
        i, t, first, last = steps[k]
        kk = st['np']
        st['np'] += 1
        tk = st['lt'].get(kk - 3)
        if tk is not None:
            mm = _pace(mm, jnp.concatenate([tk, tk], 1))
        m = mm[:, :QB]
        lo8, lo64 = _lane_lo(8), _lane_lo(64)
        if first:
            pst['l'] = pst['ll'] = pst['lu'] = None
        if t == i - 1:
            p = b_exp(Sb[slot_of[(i, 'mid')]], m, toks, st)
            pst['l'] = acc_sum(pst['l'], p)
            p2 = p.reshape(KC, QB)
            ws = [_lanes(p2, a) for a in range(4)]
        elif t == i - 2:
            ph = b_exp(Sb[slot_of[(i, 'pack')], pl.ds(0, 64), pl.ds(0, 256)], mm[:, QB:QB + 256], toks, st)
            pe = b_exp(Sb[slot_of[(i, 'edge')], pl.ds(0, 64), :], m, toks, st)
            pst['ll'] = acc_sum(None, ph)
            pst['l'] = acc_sum(pst['l'], pe)
            ph2, pe2 = ph.reshape(64, 256), pe.reshape(64, QB)
            ws = []
            for pr in range(2):
                x = _lanes(ph2, pr)
                for a, top in ((2 * pr, jnp.where(lo64, x, 0.0)), (2 * pr + 1, jnp.where(lo64, _swap(x), 0.0))):
                    ws.append(jnp.concatenate([top, _lanes(pe2, a)], 0))
        else:
            pe = b_exp(Sb[slot_of[(i, 'edge')], pl.ds(64, 64), :], m, toks, st)
            ph = b_exp(Sb[slot_of[(i, 'pack')], pl.ds(0, 64), pl.ds(256, 256)], mm[:, QB + 256:], toks, st)
            pst['lu'] = acc_sum(None, ph)
            pst['l'] = acc_sum(pst['l'], pe)
            ph2, pe2 = ph.reshape(64, 256), pe.reshape(64, QB)
            ws = []
            for pr in range(2):
                x = _lanes(ph2, pr)
                for a, bot in ((2 * pr, jnp.where(lo64, 0.0, _swap(x))), (2 * pr + 1, jnp.where(lo64, 0.0, x))):
                    ws.append(jnp.concatenate([_lanes(pe2, a), bot], 0))
        ws = [w.astype(BF) for w in ws]
        lt = pst['l']
        for extra in (pst['ll'] if t == i - 2 else None, pst['lu'] if t == i else None):
            if extra is not None:
                lt = jnp.maximum(lt, jnp.concatenate([extra, extra], 1))
        st['lt'][kk] = lt
        vrow = j * 64
        pvs = [_dot(_unpack(VTb[t, pl.ds(pl.multiple_of(vrow + 16 * a, 16), 16), :]), ws[a]) for a in range(4)]
        pst['acc'] = pvs if first else [x + y for x, y in zip(pst['acc'], pvs)]
        if last:
            l, lu, ll = pst['l'], pst['lu'], pst['ll']
            outs, invs = [], []
            for pr in range(2):
                u = _lanes(lu, pr)
                if ll is not None:
                    w_ = _lanes(ll, pr)
                    ea, eb = jnp.where(lo8, w_, _swap(u)), jnp.where(lo8, _swap(w_), u)
                else:
                    ea, eb = jnp.where(lo8, 0.0, _swap(u)), jnp.where(lo8, 0.0, u)
                for a, e in ((2 * pr, ea), (2 * pr + 1, eb)):
                    inv = 1.0 / jnp.sum(_lanes(l, a) + e, axis=0, keepdims=True)
                    outs.append(pst['acc'][a] * inv)
                    invs.append(inv)
            st['lt'][kk] = jnp.concatenate([jnp.broadcast_to(v, (8, 128)) for v in invs], 1)
            o = jnp.concatenate(outs, 0)
            OTb[i // 4, pl.ds(pl.multiple_of(vrow, 64), 64), pl.ds((i % 4) * 128, 128)] = _pack(o.astype(BF))

    def b_iter(j, jp, do_qk):
        mfin = {}
        for c in range(NCAR):
            raw = mb[c]
            if c == NCAR - 1:
                raw = b_max(raw[:, :QB], raw[:, QB:QB + 256], raw[:, QB + 256:])
            mfin[NK - NCAR + c] = raw
        toks = {}
        st = {'nt': 0, 'ne': -20 * NCAR, 'np': 0, 'lt': {}}
        pst = {}
        for n in range(NS if do_qk else B_LAG):
            if do_qk:
                i = qk_plan[n][0]
                if n == 0 or qk_plan[n - 1][0] != i:
                    st['cm'] = st['cl'] = st['cu'] = None
                b_qk(j, n, st, toks)
                if n == NS - 1 or qk_plan[n + 1][0] != i:
                    if i == NK - 1:
                        mb[NCAR - 1] = jnp.concatenate([st['cm'], st['cl'], st['cu']], 1)
                    elif i >= NK - NCAR:
                        mb[i - (NK - NCAR)] = b_max(st['cm'], st['cl'], st['cu'])
                    else:
                        mfin[i] = b_max(st['cm'], st['cl'], st['cu'])
            k = n - B_LAG
            if k >= 0:
                b_pv(j, k, mfin[steps[k][0]], pst, toks, st)
            else:
                b_pv(jp, k + NS, mfin[steps[k + NS][0]], pst, toks, st)

    def b_body(j, carry):
        b_iter(j, jnp.maximum(j - 1, 0), True)
        return carry
    lax.fori_loop(0, D // 128, b_body, 0)

    for n, (r0, nr) in enumerate(ob_blocks):
        qb, off = divmod(r0, QB)
        r = lax.dot_general(_unpack(OTb[qb, :, pl.ds(off, nr)]), wob[...], TN_DIMS, preferred_element_type=F32)
        if n == 0:
            b_iter(None, D // 128 - 1, False)
        ob[pl.ds(r0, nr), :] = r.astype(BF)
        ob_cp(r0, nr, n).start()

    for qb in range(S // QB):
        oa_cp(qb).wait()
    for n, (r0, nr) in enumerate(ob_blocks):
        ob_cp(r0, nr, n).wait()


@jax.jit
def pallas_concat_heads__grouped_kv_mqa__sliding_block__prompt_kernel(
        A_x, A_wq, A_wk, A_wv, A_wo, B_x, B_wqkv, B_wo):
    vm = pltpu.VMEM
    scratch = [
        vm((S, D), BF), vm((S, D), BF),
        vm((D, D), BF), vm((D, D), BF),
        vm((D, 3 * D), BF), vm((D, D), BF),
        vm((D + 2 * DH, D), BF), vm((2 * D, D), BF),
        vm((S // QB, D // 2, QB), I32),
        vm((NK, DH // 2, KC), I32),
        vm((S // 2, DH), I32),
        vm((S // QB, D // 2, QB), I32),
        vm((S, QB), F32), vm((S, QB), F32),
        vm((8, QB), F32), vm((8, QB), F32),
        vm((NK, D // 2, KC), I32), vm((NK, D // 2, KC), I32),
        vm((D // 128, S // 2, 128), I32),
        vm((S // QB, D // 2, QB), I32),
        vm((B_RING, KC, QB), F32),
        vm((B_LAG // 3, 8, 2 * QB), F32),
        vm((S, D), BF), vm((S, D), BF),
        vm((KC, 128), I32), vm((64, 128), I32),
        pltpu.SemaphoreType.DMA((56,)),
    ]
    hbm = pl.BlockSpec(memory_space=pltpu.HBM)
    return pl.pallas_call(
        _kernel,
        out_shape=jax.ShapeDtypeStruct((1, S, 2 * D), BF),
        in_specs=[hbm] * 8,
        out_specs=hbm,
        scratch_shapes=scratch,
        compiler_params=pltpu.CompilerParams(vmem_limit_bytes=120 * 2**20),
        name="fused",
    )(A_x, A_wq, A_wk.T, A_wv.T, A_wo, B_x, B_wqkv, B_wo)
```
